```python
import jax
import jax.numpy as jnp

def _softmax(x, axis=-1):
    return jax.nn.softmax(x, axis=axis)
def _gelu(x):
    return jax.nn.gelu(x, approximate=True)
def _silu(x):
    return jax.nn.silu(x)
def _sigmoid(x):
    return jax.nn.sigmoid(x)
def _layernorm(x, axis=-1, eps=1e-5):
    m = jnp.mean(x, axis=axis, keepdims=True)
    v = jnp.var(x, axis=axis, keepdims=True)
    return (x - m) / jnp.sqrt(v + eps)
def _scatter_add(tgt, idx, src, axis=0):
    return tgt.at[idx].add(src)
def _segment_sum(src, seg, n):
    return jax.ops.segment_sum(src, seg, n)
class _Rng:
    def __init__(self, key):
        self._k = key
    def _next(self):
        self._k, sub = jax.random.split(self._k)
        return sub
    def normal(self, shape):
        return jax.random.normal(self._next(), shape, dtype=jnp.bfloat16)
    def randint(self, lo, hi, shape):
        return jax.random.randint(self._next(), shape, lo, hi, dtype=jnp.int32)
    def uniform(self, shape, lo=0.0, hi=1.0):
        return jax.random.uniform(self._next(), shape, jnp.bfloat16, lo, hi)
    def permutation(self, n):
        return jax.random.permutation(self._next(), n)


kernel_name = 'standalone__cross_network_dcn__recsys'

def setup_inputs():
    _rng = _Rng(jax.random.key(int.from_bytes(__import__("os").urandom(4), "little")))
    _w = (lambda a: (lambda t: t.astype(jnp.bfloat16) if jnp.issubdtype(t.dtype, jnp.floating) else t)(jnp.asarray(a)))
    B, F, D, L = 16384, 100, 16, 6
    Din = min(F * D, 1024)
    return {
        "x0": _w((lambda *s: _rng.normal(s) * 0.05)(B, Din)),
        "ws": _w((lambda *s: _rng.normal(s) * 0.05)(L, Din, Din) * (Din ** -0.5)),
        "bs": _w((lambda *s: _rng.normal(s) * 0.05)(L, Din) * 0.01),
    }

def reference(x0, ws, bs):
    x = x0
    L = ws.shape[0]
    for l in range(L):
        proj = jnp.einsum('bd,de->be', x, ws[l]) + bs[l]
        x = x0 * proj + x
    return x
```

```python
import jax
import jax.numpy as jnp
import jax.experimental.pallas as pl
import jax.experimental.pallas.tpu as pltpu


def _kernel(x0_ref, ws_ref, bs_ref, o_ref):
    x0 = x0_ref[...].astype(jnp.float32)
    x = x0
    xb = x0_ref[...]
    for l in range(ws_ref.shape[0]):
        p = jnp.dot(xb, ws_ref[l], preferred_element_type=jnp.float32)
        p = p + bs_ref[l:l + 1, :].astype(jnp.float32)
        x = x0 * p + x
        xb = x.astype(o_ref.dtype)
    o_ref[...] = xb


@jax.jit
def pallas_standalone__cross_network_dcn__recsys_kernel(x0, ws, bs):
    B, D = x0.shape
    L = ws.shape[0]
    tm = 512
    return pl.pallas_call(
        _kernel,
        grid=(B // tm,),
        in_specs=[
            pl.BlockSpec((tm, D), lambda i: (i, 0)),
            pl.BlockSpec((L, D, D), lambda i: (0, 0, 0), pipeline_mode=pl.Buffered(1)),
            pl.BlockSpec((L, D), lambda i: (0, 0)),
        ],
        out_specs=pl.BlockSpec((tm, D), lambda i: (i, 0)),
        out_shape=jax.ShapeDtypeStruct((B, D), x0.dtype),
        compiler_params=pltpu.CompilerParams(
            dimension_semantics=("parallel",), vmem_limit_bytes=100 * 2**20),
    )(x0, ws, bs)
```

```python
import numpy as np
import jax
import jax.numpy as jnp
import jax.experimental.pallas as pl
import jax.experimental.pallas.tpu as pltpu

F32, BF16 = jnp.float32, jnp.bfloat16

_SA = {1: [(1, (0, 0)), (1, (1, 1))], 2: [(1, (1, 0)), (1, (1, 1))], 3: [(1, (0, 0))],
       4: [(1, (1, 1))], 5: [(1, (0, 0)), (1, (0, 1))], 6: [(1, (1, 0)), (-1, (0, 0))],
       7: [(1, (0, 1)), (-1, (1, 1))]}
_SB = {1: [(1, (0, 0)), (1, (1, 1))], 2: [(1, (0, 0))], 3: [(1, (0, 1)), (-1, (1, 1))],
       4: [(1, (1, 0)), (-1, (0, 0))], 5: [(1, (1, 1))], 6: [(1, (0, 0)), (1, (0, 1))],
       7: [(1, (1, 0)), (1, (1, 1))]}
_SC = {1: [(1, (0, 0)), (1, (1, 1))], 2: [(1, (1, 0)), (-1, (1, 1))],
       3: [(1, (0, 1)), (1, (1, 1))], 4: [(1, (0, 0)), (1, (1, 0))],
       5: [(-1, (0, 0)), (1, (0, 1))], 6: [(1, (1, 1))], 7: [(1, (0, 0))]}
_NTERMS = {(0, 0): 4, (0, 1): 2, (1, 0): 2, (1, 1): 4}
_QUAD = [(0, 0), (0, 1), (1, 0), (1, 1)]
_BLOCKS = [(i, j) for i in range(4) for j in range(4)]
_ORDERS = ([3, 5, 6, 1, 2, 4, 7], [4, 2, 7, 1, 5, 3, 6])
_TM = 512
_DELAY = 3


def _sub(q, k):
    return (2 * q[0] + k[0], 2 * q[1] + k[1])


def _comb(terms, get):
    out = get(terms[0][1])
    for sign, key in terms[1:]:
        out = out + get(key) if sign > 0 else out - get(key)
    return out


class _Sum:
    def __init__(self, init=None):
        self.v, self.sign, self.n = init, 1, 0

    def add(self, sign, v):
        self.n += 1
        if self.v is None:
            self.v, self.sign = v, sign
        elif sign == self.sign:
            self.v = self.v + v
        elif self.sign > 0:
            self.v = self.v - v
        else:
            self.v, self.sign = v - self.v, 1


def _kernel(zero_ref, x0_ref, ws_hbm, bs_ref, o_ref, wt_ref, w_ref, b_ref, x_ref, sem):
    L, D, _ = ws_hbm.shape
    s, r = D // 4, x0_ref.shape[0] // 4
    wt = wt_ref.bitcast(BF16)
    always = zero_ref[0] == 0

    def blk(ref, ij):
        return ref.at[ij[0] * r:(ij[0] + 1) * r, ij[1] * s:(ij[1] + 1) * s]

    def layer(l, x, order, pending, clock, emit):
        out = {}
        c = {ij: _Sum(b_ref[l, :, ij[1] * s:(ij[1] + 1) * s]) for ij in _BLOCKS}
        for p in order:
            ap = {k: _comb(_SA[p], lambda q: x[_sub(q, k)]) for k in _QUAD}
            m = {k: _Sum() for k in _QUAD}
            for q in order:
                a = _comb(_SA[q], ap.get)
                clock[0] += 1
                if pending and pending[0][0] + _DELAY <= clock[0]:
                    a = jnp.where(always, a, pending.pop(0)[1])
                prod = jnp.dot(a.astype(BF16), wt[l * 49 + (p - 1) * 7 + q - 1],
                               preferred_element_type=F32)
                for sign, k in _SC[q]:
                    m[k].add(sign, prod)
                    if m[k].n < _NTERMS[k]:
                        continue
                    for sign2, quad in _SC[p]:
                        ij = _sub(quad, k)
                        c[ij].add(sign2 * m[k].sign, m[k].v)
                        v = c[ij].v
                        if c[ij].n == _NTERMS[quad]:
                            v = out[ij] = blk(x0_ref, ij)[...].astype(F32) * v + x[ij]
                            emit(ij, v)
                        pending.append((clock[0], v))
        return out

    def w_copy(l):
        return pltpu.make_async_copy(ws_hbm.at[l], w_ref.at[l], sem.at[l])

    def w_sums(l):
        def body(i, carry):
            r0 = pl.multiple_of(i * 16, 16)
            w = {ij: w_ref[l, pl.ds(ij[0] * s + r0, 16), pl.ds(ij[1] * s, s)].astype(F32)
                 for ij in _BLOCKS}
            for p in range(1, 8):
                bp = {k: _comb(_SB[p], lambda q: w[_sub(q, k)]) for k in _QUAD}
                for q in range(1, 8):
                    wt[l * 49 + (p - 1) * 7 + q - 1, pl.ds(r0, 16), :] = (
                        _comb(_SB[q], bp.get).astype(BF16))
            return carry
        jax.lax.fori_loop(0, s // 16, body, 0)

    @pl.when(pl.program_id(0) == 0)
    def _():
        for l in range(L):
            w_copy(l).start()
        for l in range(L):
            b_ref[l] = bs_ref[l:l + 1, :].astype(F32)
        x_ref[...] = x0_ref[...].astype(F32)

        def body(l, carry):
            w_copy(l).wait()
            w_sums(l)

            def emit(ij, v):
                blk(x_ref, ij)[...] = v
            layer(l, {ij: blk(x_ref, ij)[...] for ij in _BLOCKS}, _ORDERS[0], [], [0], emit)
            return carry
        jax.lax.fori_loop(0, L, body, 0)
        o_ref[...] = x_ref[...].astype(o_ref.dtype)

    @pl.when(pl.program_id(0) > 0)
    def _():
        x = {ij: blk(x0_ref, ij)[...].astype(F32) for ij in _BLOCKS}
        pending, clock = [], [0]
        for l in range(L):
            def emit(ij, v, last=l == L - 1):
                if last:
                    blk(o_ref, ij)[...] = v.astype(o_ref.dtype)
            x = layer(l, x, _ORDERS[l % 2], pending, clock, emit)


@jax.jit
def pallas_standalone__cross_network_dcn__recsys_kernel(x0, ws, bs):
    B, D = x0.shape
    L = ws.shape[0]
    s = D // 4
    return pl.pallas_call(
        _kernel,
        grid=(B // _TM,),
        in_specs=[
            pl.BlockSpec(memory_space=pltpu.SMEM),
            pl.BlockSpec((_TM, D), lambda i: (i, 0)),
            pl.BlockSpec(memory_space=pl.ANY),
            pl.BlockSpec((L, D), lambda i: (0, 0)),
        ],
        out_specs=pl.BlockSpec((_TM, D), lambda i: (i, 0)),
        out_shape=jax.ShapeDtypeStruct((B, D), x0.dtype),
        scratch_shapes=[
            pltpu.VMEM((L * 49, s // 2, s), jnp.uint32),
            pltpu.VMEM((L, D, D), ws.dtype),
            pltpu.VMEM((L, 1, D), F32),
            pltpu.VMEM((_TM, D), F32),
            pltpu.SemaphoreType.DMA((L,)),
        ],
        compiler_params=pltpu.CompilerParams(
            dimension_semantics=("arbitrary",), vmem_limit_bytes=100 * 2**20),
    )(np.zeros((1,), np.int32), x0, ws, bs)
```

```python
import jax
import jax.numpy as jnp
import jax.experimental.pallas as pl
import jax.experimental.pallas.tpu as pltpu

F32, BF16 = jnp.float32, jnp.bfloat16

_SA = {1: [(1, (0, 0)), (1, (1, 1))], 2: [(1, (1, 0)), (1, (1, 1))], 3: [(1, (0, 0))],
       4: [(1, (1, 1))], 5: [(1, (0, 0)), (1, (0, 1))], 6: [(1, (1, 0)), (-1, (0, 0))],
       7: [(1, (0, 1)), (-1, (1, 1))]}
_SB = {1: [(1, (0, 0)), (1, (1, 1))], 2: [(1, (0, 0))], 3: [(1, (0, 1)), (-1, (1, 1))],
       4: [(1, (1, 0)), (-1, (0, 0))], 5: [(1, (1, 1))], 6: [(1, (0, 0)), (1, (0, 1))],
       7: [(1, (1, 0)), (1, (1, 1))]}
_SC = {1: [(1, (0, 0)), (1, (1, 1))], 2: [(1, (1, 0)), (-1, (1, 1))],
       3: [(1, (0, 1)), (1, (1, 1))], 4: [(1, (0, 0)), (1, (1, 0))],
       5: [(-1, (0, 0)), (1, (0, 1))], 6: [(1, (1, 1))], 7: [(1, (0, 0))]}
_NTERMS = {(0, 0): 4, (0, 1): 2, (1, 0): 2, (1, 1): 4}
_QUAD = [(0, 0), (0, 1), (1, 0), (1, 1)]
_BLOCKS = [(i, j) for i in range(4) for j in range(4)]
_ORDERS = ([3, 5, 6, 1, 2, 4, 7], [4, 2, 7, 1, 5, 3, 6])
_HEAD = 256
_TM = 576
_DELAY = 4
_W_AHEAD = 2


def _sub(q, k):
    return (2 * q[0] + k[0], 2 * q[1] + k[1])


def _comb(terms, get):
    out = get(terms[0][1])
    for sign, key in terms[1:]:
        out = out + get(key) if sign > 0 else out - get(key)
    return out


class _Sum:
    def __init__(self, init=None):
        self.v, self.sign, self.n = init, 1, 0

    def add(self, sign, v):
        self.n += 1
        if self.v is None:
            self.v, self.sign = v, sign
        elif sign == self.sign:
            self.v = self.v + v
        elif self.sign > 0:
            self.v = self.v - v
        else:
            self.v, self.sign = v - self.v, 1


def _kernel(x0_hbm, ws_hbm, bs_hbm, o_hbm, wsum_ref, w_ref, bs_ref, b_ref, hx0_ref, hx_ref,
            hxb_ref, in_ref, out_ref, zero_ref, w_sem, in_sem, out_sem):
    L, D, _ = ws_hbm.shape
    tm, head = in_ref.shape[1], hx_ref.shape[0]
    n_tiles = (x0_hbm.shape[0] - head) // tm
    s, r = D // 4, tm // 4

    def cols(j):
        return slice(j * s, (j + 1) * s)

    def w_index(l, p, q):
        return l * 49 + (p - 1) * 7 + q - 1

    def always(rows):
        return jnp.tile(zero_ref[...], (rows // 8, s // 128)) == 0

    def w_copy(l):
        return pltpu.make_async_copy(ws_hbm.at[l], w_ref.at[l], w_sem.at[l])

    def in_copy(t):
        return pltpu.make_async_copy(
            x0_hbm.at[pl.ds(head + t * tm, tm)], in_ref.at[t % 2], in_sem.at[t % 2])

    def out_copy(t):
        return pltpu.make_async_copy(
            out_ref.at[t % 2], o_hbm.at[pl.ds(head + t * tm, tm)], out_sem.at[t % 2])

    head_in = pltpu.make_async_copy(x0_hbm.at[pl.ds(0, head)], hx0_ref, in_sem.at[2])
    bias_in = pltpu.make_async_copy(bs_hbm, bs_ref, in_sem.at[3])
    head_out = pltpu.make_async_copy(hxb_ref, o_hbm.at[pl.ds(0, head)], out_sem.at[2])

    head_in.start()
    bias_in.start()
    w_copy(0).start()
    zero_ref[...] = jnp.zeros(zero_ref.shape, zero_ref.dtype)
    head_in.wait()
    bias_in.wait()
    for l in range(L):
        b_ref[l] = bs_ref[l:l + 1, :].astype(F32)
    hxb_ref[...] = hx0_ref[...]
    hx_ref[...] = hx0_ref[...].astype(F32)

    def head_layer(l, carry):
        w_copy(l).wait()

        @pl.when(l == 0)
        def _():
            for k in range(1, _W_AHEAD):
                w_copy(k).start()

        @pl.when(l + _W_AHEAD < L)
        def _():
            w_copy(l + _W_AHEAD).start()

        @pl.when(l + _W_AHEAD == L)
        def _():
            in_copy(0).start()

        xb = hxb_ref[...]
        partial = []
        for j in range(4):
            acc = b_ref[l, :, cols(j)]
            for i in range(4):
                acc = acc + jnp.dot(xb[:, cols(i)], w_ref[l, cols(i), cols(j)],
                                    preferred_element_type=F32)
                partial.append(acc)
            x = hx0_ref[:, cols(j)].astype(F32) * acc + hx_ref[:, cols(j)]
            hx_ref[:, cols(j)] = x
            hxb_ref[:, cols(j)] = x.astype(BF16)

        keep = always(16)
        groups = head // 16
        for n in range(s // 16):
            w = {}
            for k, (i, j) in enumerate(_BLOCKS):
                g = (n * 16 + k) * (len(partial) - 1) * groups // s
                w[i, j] = jnp.where(
                    keep, w_ref[l, pl.ds(i * s + n * 16, 16), cols(j)].astype(F32),
                    partial[g // groups][g % groups * 16:g % groups * 16 + 16])
            for p in range(1, 8):
                bp = {k: _comb(_SB[p], lambda q: w[_sub(q, k)]) for k in _QUAD}
                for q in range(1, 8):
                    wsum_ref[w_index(l, p, q), pl.ds(n * 16, 16), :] = (
                        _comb(_SB[q], bp.get).astype(BF16))
        return carry

    jax.lax.fori_loop(0, L, head_layer, 0)
    head_out.start()

    def tile(t, carry):
        @pl.when(t + 1 < n_tiles)
        def _():
            in_copy(t + 1).start()

        in_copy(t).wait()

        @pl.when(t >= 2)
        def _():
            out_copy(t - 2).wait()

        def blk(ref, ij):
            return ref.at[t % 2, ij[0] * r:(ij[0] + 1) * r, cols(ij[1])]

        keep = always(r)
        x = {ij: blk(in_ref, ij)[...].astype(F32) for ij in _BLOCKS}
        pending, clock = [], 0
        for l in range(L):
            order = _ORDERS[l % 2]
            x_next = {}
            c = {ij: _Sum(b_ref[l, :, cols(ij[1])]) for ij in _BLOCKS}
            for p in order:
                ap = {k: _comb(_SA[p], lambda q: x[_sub(q, k)]) for k in _QUAD}
                m = {k: _Sum() for k in _QUAD}
                for q in order:
                    a = _comb(_SA[q], ap.get)
                    clock += 1
                    if pending and pending[0][0] + _DELAY <= clock:
                        a = jnp.where(keep, a, pending.pop(0)[1])
                    prod = jnp.dot(a.astype(BF16), wsum_ref[w_index(l, p, q)],
                                   preferred_element_type=F32)
                    for sign, k in _SC[q]:
                        m[k].add(sign, prod)
                        if m[k].n < _NTERMS[k]:
                            continue
                        for sign2, quad in _SC[p]:
                            ij = _sub(quad, k)
                            c[ij].add(sign2 * m[k].sign, m[k].v)
                            v = c[ij].v
                            if c[ij].n == _NTERMS[quad]:
                                v = blk(in_ref, ij)[...].astype(F32) * v + x[ij]
                                x_next[ij] = v
                                if l == L - 1:
                                    blk(out_ref, ij)[...] = v.astype(BF16)
                            pending.append((clock, v))
            x = x_next
        out_copy(t).start()
        return carry

    jax.lax.fori_loop(0, n_tiles, tile, 0)
    head_out.wait()
    for t in range(max(n_tiles - 2, 0), n_tiles):
        out_copy(t).wait()


@jax.jit
def pallas_standalone__cross_network_dcn__recsys_kernel(x0, ws, bs):
    B, D = x0.shape
    L = ws.shape[0]
    s = D // 4
    assert B > _HEAD and (B - _HEAD) % _TM == 0 and s % 128 == 0 and L >= _W_AHEAD
    assert x0.dtype == ws.dtype == bs.dtype == BF16
    hbm = pl.BlockSpec(memory_space=pl.ANY)
    return pl.pallas_call(
        _kernel,
        in_specs=[hbm, hbm, hbm],
        out_specs=hbm,
        out_shape=jax.ShapeDtypeStruct((B, D), BF16),
        scratch_shapes=[
            pltpu.VMEM((L * 49, s, s), BF16),
            pltpu.VMEM((L, D, D), BF16),
            pltpu.VMEM((L, D), BF16),
            pltpu.VMEM((L, 1, D), F32),
            pltpu.VMEM((_HEAD, D), BF16),
            pltpu.VMEM((_HEAD, D), F32),
            pltpu.VMEM((_HEAD, D), BF16),
            pltpu.VMEM((2, _TM, D), BF16),
            pltpu.VMEM((2, _TM, D), BF16),
            pltpu.VMEM((8, 128), jnp.int32),
            pltpu.SemaphoreType.DMA((L,)),
            pltpu.SemaphoreType.DMA((4,)),
            pltpu.SemaphoreType.DMA((3,)),
        ],
        compiler_params=pltpu.CompilerParams(
            vmem_limit_bytes=100 * 2**20, disable_bounds_checks=True),
    )(x0, ws, bs)
```
